```python
import jax
import jax.numpy as jnp

def _softmax(x, axis=-1):
    return jax.nn.softmax(x, axis=axis)

def _gelu(x):
    return jax.nn.gelu(x, approximate=True)

def _silu(x):
    return jax.nn.silu(x)

def _sigmoid(x):
    return jax.nn.sigmoid(x)

def _layernorm(x, axis=-1, eps=1e-05):
    m = jnp.mean(x, axis=axis, keepdims=True)
    v = jnp.var(x, axis=axis, keepdims=True)
    return (x - m) / jnp.sqrt(v + eps)

def _scatter_add(tgt, idx, src, axis=0):
    return tgt.at[idx].add(src)

def _segment_sum(src, seg, n):
    return jax.ops.segment_sum(src, seg, n)

class _Rng:

    def __init__(self, key):
        self._k = key

    def _next(self):
        self._k, sub = jax.random.split(self._k)
        return sub

    def normal(self, shape):
        return jax.random.normal(self._next(), shape, dtype=jnp.bfloat16)

    def randint(self, lo, hi, shape):
        return jax.random.randint(self._next(), shape, lo, hi, dtype=jnp.int32)

    def uniform(self, shape, lo=0.0, hi=1.0):
        return jax.random.uniform(self._next(), shape, jnp.bfloat16, lo, hi)

    def permutation(self, n):
        return jax.random.permutation(self._next(), n)
kernel_name = 'concat_heads__compressed_kv_cla__memory_aug_recurrent_mem_tr__prompt'

def setup_inputs():
    _rng = _Rng(jax.random.key(int.from_bytes(__import__("os").urandom(4), "little")))
    _w = lambda a: (lambda t: t.astype(jnp.bfloat16) if jnp.issubdtype(t.dtype, jnp.floating) else t)(jnp.asarray(a))

    def _A_setup():
        B, H, Sq, Sk, D, M = (1, 32, 2048, 2048, 128, 576)
        Dc = 4 * D
        return {'x': _w((lambda *s: _rng.normal(s) * 0.05)(B, Sq, M)), 'c_kv': _w((lambda *s: _rng.normal(s) * 0.05)(B, Sk, Dc)), 'w_q': _w((lambda *s: _rng.normal(s) * 0.05)(M, H, D) * M ** (-0.5)), 'w_uk': _w((lambda *s: _rng.normal(s) * 0.05)(Dc, H, D) * Dc ** (-0.5)), 'w_uv': _w((lambda *s: _rng.normal(s) * 0.05)(Dc, H, D) * Dc ** (-0.5)), 'w_o': _w((lambda *s: _rng.normal(s) * 0.05)(H, D, M) * (H * D) ** (-0.5))}
    _A_in = _A_setup()

    def _B_setup():
        B, S, Dm = (1, 2048, 576)
        H, Dh = (32, 128)
        M, seg = (8, 32)
        seg = min(seg, S)
        S = S // seg * seg
        return {'x': _w((lambda *s: _rng.normal(s) * 0.05)(B, S, Dm)), 'mem0': _w((lambda *s: _rng.normal(s) * 0.05)(B, M, Dm)), 'Wq': _w((lambda *s: _rng.normal(s) * 0.05)(Dm, H, Dh) * Dm ** (-0.5)), 'Wk': _w((lambda *s: _rng.normal(s) * 0.05)(Dm, H, Dh) * Dm ** (-0.5)), 'Wv': _w((lambda *s: _rng.normal(s) * 0.05)(Dm, H, Dh) * Dm ** (-0.5)), 'Wo': _w((lambda *s: _rng.normal(s) * 0.05)(H, Dh, Dm) * (H * Dh) ** (-0.5)), 'seg_len': seg}
    _B_in = _B_setup()
    return {'A_x': _A_in['x'], 'A_c_kv': _A_in['c_kv'], 'A_w_q': _A_in['w_q'], 'A_w_uk': _A_in['w_uk'], 'A_w_uv': _A_in['w_uv'], 'A_w_o': _A_in['w_o'], 'B_x': _B_in['x'], 'B_mem0': _B_in['mem0'], 'B_Wq': _B_in['Wq'], 'B_Wk': _B_in['Wk'], 'B_Wv': _B_in['Wv'], 'B_Wo': _B_in['Wo'], 'B_seg_len': _B_in['seg_len']}

def reference(A_x, A_c_kv, A_w_q, A_w_uk, A_w_uv, A_w_o, B_x, B_mem0, B_Wq, B_Wk, B_Wv, B_Wo, B_seg_len):

    def _A_ref(x, c_kv, w_q, w_uk, w_uv, w_o):
        B, Sq, M = (x.shape[0], x.shape[1], x.shape[2])
        Sk = c_kv.shape[1]
        H, D = (w_q.shape[1], w_q.shape[2])
        q = jnp.einsum('bqm,mhd->bhqd', x, w_q)
        k = jnp.einsum('bkc,chd->bhkd', c_kv, w_uk)
        v = jnp.einsum('bkc,chd->bhkd', c_kv, w_uv)
        scores = jnp.einsum('bhqd,bhkd->bhqk', q, k) * D ** (-0.5)
        off = Sk - Sq
        qi = jnp.arange(Sq)[:, None]
        kj = jnp.arange(Sk)[None, :]
        cmask = kj <= qi + off
        scores = jnp.where(cmask[None, None], scores, -1000000000.0)
        p = _softmax(scores, axis=-1)
        ctx = jnp.einsum('bhqk,bhkd->bhqd', p, v)
        return jnp.einsum('bhqd,hdm->bqm', ctx, w_o)

    def _B_ref(x, mem0, Wq, Wk, Wv, Wo, seg_len):
        B, S, Dm = x.shape
        H, Dh = (Wq.shape[1], Wq.shape[2])
        M = mem0.shape[1]
        scale = Dh ** (-0.5)
        n_seg = S // seg_len
        L = M + seg_len
        idx = jnp.arange(L)
        mask = (idx[:, None] < M) | (idx[:, None] >= idx[None, :])
        mem = mem0
        outs = []
        for s in range(n_seg):
            xs = x[:, s * seg_len:(s + 1) * seg_len, :].copy()
            h = jnp.concatenate([mem, xs], axis=1)
            q = jnp.einsum('btd,dhe->bhte', h, Wq)
            k = jnp.einsum('btd,dhe->bhte', h, Wk)
            v = jnp.einsum('btd,dhe->bhte', h, Wv)
            scores = jnp.einsum('bhqe,bhke->bhqk', q, k) * scale
            scores = jnp.where(mask[None, None], scores, -1000000000.0)
            p = _softmax(scores, axis=-1)
            o = jnp.einsum('bhqk,bhke->bhqe', p, v)
            o = jnp.einsum('bhte,hed->btd', o, Wo)
            mem = o[:, :M, :].copy()
            outs.append(o[:, M:, :])
        return jnp.concatenate(outs, axis=1)
    a = _A_ref(A_x, A_c_kv, A_w_q, A_w_uk, A_w_uv, A_w_o)
    b = _B_ref(B_x, B_mem0, B_Wq, B_Wk, B_Wv, B_Wo, B_seg_len)
    return jnp.concatenate([a, b], axis=-1)
```

```python
import functools
import numpy as np
import jax
import jax.numpy as jnp
from jax import lax
from jax.experimental import pallas as pl
from jax.experimental.pallas import tpu as pltpu

S = 2048; DM = 576; DC = 512; H = 32; D = 128; NM = 8; SEG = 32
NSEG = S // SEG
LOG2E = float(np.log2(np.e))
SCALE = float(D ** -0.5) * LOG2E
bf16 = jnp.bfloat16; f32 = jnp.float32; u32 = jnp.uint32
NT = (((1,), (1,)), ((), ()))
B_AHEAD = 2; B_LAG = 4; B_G = 4
A_PCH = 128
A_QKA = 0

def repack(ev, od):
    lo = (ev & u32(0xffff)) | (od << 16)
    hi = (ev >> 16) | (od & u32(0xffff0000))
    return lo, hi

def kernel(xa_h, c_h, wq_h, wuk_h, wuv_h, woa_h, xb_h, mem_h, bq_h, bk_h, bv_h, wob_h, out_h,
           xt_s, xa_s, c_s, xb_s, mem_s, woa_s, wob_s, uq, uk, uv, ubq, ubk, ubv,
           wq_p, wkv_p, wb, acc, out_s, q_s, k_s, v_s, sem_a, sem_b, sem_m, sem_o, *, do_a, do_b):
    m_c = pltpu.make_async_copy(c_h, c_s, sem_m.at[0])
    m_xa = pltpu.make_async_copy(xa_h, xt_s.at[0], sem_m.at[1])
    m_woa = pltpu.make_async_copy(woa_h.bitcast(u32), woa_s, sem_m.at[2])
    m_xb = pltpu.make_async_copy(xb_h, xt_s.at[1], sem_m.at[3])
    m_mem = pltpu.make_async_copy(mem_h, mem_s, sem_m.at[4])
    m_wob = pltpu.make_async_copy(wob_h.bitcast(u32), wob_s, sem_m.at[5])
    rq, rk, rv = wq_h.bitcast(u32), wuk_h.bitcast(u32), wuv_h.bitcast(u32)
    sq, sk, sv = bq_h.bitcast(u32), bk_h.bitcast(u32), bv_h.bitcast(u32)
    def a_cp(i, j):
        src = (rk, rv, rq)[i]; dst = (uk, uv, uq)[i]
        return pltpu.make_async_copy(src.at[:, j, :], dst.at[j], sem_a.at[i, j])
    def b_cp(i, j):
        src = (sq, sk, sv)[i]; dst = (ubq, ubk, ubv)[i]
        return pltpu.make_async_copy(src.at[:, j, :], dst.at[j], sem_b.at[i, j])
    m_xa.start()
    m_c.start()
    for i in range(3): a_cp(i, 0).start()
    m_woa.start()
    for j in range(1, 16):
        for i in range(3): a_cp(i, j).start()
    m_xb.start()
    for j in range(16):
        for i in range(3): b_cp(i, j).start()
    m_mem.start(); m_wob.start()

    acc[...] = jnp.zeros(acc.shape, f32)
    m_xa.wait()
    for t in range(4):
        xa_s[t * 512:(t + 1) * 512, :] = xt_s[0, :, t * 512:(t + 1) * 512].T
    m_c.wait(); m_woa.wait()
    row = lax.broadcasted_iota(jnp.int32, (128, 128), 0)
    col = lax.broadcasted_iota(jnp.int32, (128, 128), 1)
    tri = row >= col

    def prep_w(j):
        sl = j % 2
        for i in range(3):
            a_cp(i, j).wait()
        lo, hi = repack(uq[j, pl.ds(0, DM // 2, stride=2), :], uq[j, pl.ds(1, DM // 2, stride=2), :])
        wq_p[sl, 0] = lo; wq_p[sl, 1] = hi
        lo, hi = repack(uk[j, pl.ds(0, DC // 2, stride=2), :], uk[j, pl.ds(1, DC // 2, stride=2), :])
        wkv_p[sl, 0, :, 0:128] = lo; wkv_p[sl, 1, :, 0:128] = hi
        lo, hi = repack(uv[j, pl.ds(0, DC // 2, stride=2), :], uv[j, pl.ds(1, DC // 2, stride=2), :])
        wkv_p[sl, 0, :, 128:256] = lo; wkv_p[sl, 1, :, 128:256] = hi

    def proj(sl, hh, r0, n):
        wq = pltpu.bitcast(wq_p[sl, hh], bf16)
        wkv = pltpu.bitcast(wkv_p[sl, hh], bf16)
        kv = jnp.dot(c_s[r0:r0 + n, :], wkv, preferred_element_type=f32)
        k_s[hh, r0:r0 + n, :] = kv[:, 0:128].astype(bf16)
        v_s[hh, r0:r0 + n, :] = kv[:, 128:256].astype(bf16)
        q = jnp.dot(xa_s[r0:r0 + n, :], wq, preferred_element_type=f32) * SCALE
        q_s[hh, r0:r0 + n, :] = q.astype(bf16)

    def qk(hh, qi):
        n = (qi + 1) * 128
        return lax.dot_general(q_s[hh, qi * 128:n, :], k_s[hh, 0:n, :], NT, preferred_element_type=f32)

    def sm_pv(hh, qi, s):
        n = (qi + 1) * 128
        sd = jnp.where(tri, s[:, n - 128:], -1e30)
        s = jnp.concatenate([s[:, :n - 128], sd], axis=1) if qi > 0 else sd
        m = jnp.max(s, axis=1, keepdims=True)
        p = jnp.exp2(s - m)
        l = jnp.sum(p, axis=1, keepdims=True)
        o = jnp.dot(p.astype(bf16), v_s[hh, 0:n, :], preferred_element_type=f32)
        return (o * (1.0 / l)).astype(bf16)

    def oproj(h, qi, ctx):
        w = pltpu.bitcast(woa_s[pl.ds(pl.multiple_of(h * (DM // 2), DM // 2), DM // 2), :], bf16)
        acc[qi * 128:(qi + 1) * 128, :] += lax.dot_general(ctx, w, NT, preferred_element_type=f32)

    prep_w(0)
    proj(0, 0, 0, S)

    def pair_body(j, carry):
        sl = j % 2
        jn = jnp.minimum(j + 1, 15)
        @pl.when(j < 15)
        def _():
            prep_w(j + 1)
        nch = S // A_PCH; every = 16 // nch
        for hh in range(2):
            h = 2 * j + hh
            nsl = sl if hh == 0 else jn % 2
            nh = 1 - hh
            s_cur = qk(hh, 0)
            prev = None
            for qi in range(16):
                if A_QKA and qi < 15:
                    s_next = qk(hh, qi + 1)
                if qi % every == 0:
                    proj(nsl, nh, (qi // every) * A_PCH, A_PCH)
                ctx = sm_pv(hh, qi, s_cur)
                if prev is not None:
                    oproj(h, qi - 1, prev)
                prev = ctx
                if qi < 15:
                    s_cur = s_next if A_QKA else qk(hh, qi + 1)
            oproj(h, 15, prev)
        return carry
    if do_a:
        lax.fori_loop(0, 16, pair_body, 0)
    else:
        for j in range(1, 16):
            for i in range(3): a_cp(i, j).wait()
    out_s[:, 0:DM] = acc[...].astype(bf16)

    m_xb.wait()
    for t in range(4):
        xb_s[t * 512:(t + 1) * 512, :] = xt_s[1, :, t * 512:(t + 1) * 512].T
    for j in range(16):
        for i, u in enumerate((ubq, ubk, ubv)):
            b_cp(i, j).wait()
            lo, hi = repack(u[j, pl.ds(0, DM // 2, stride=2), :], u[j, pl.ds(1, DM // 2, stride=2), :])
            wb[:, (2 * j) * 384 + i * 128:(2 * j) * 384 + (i + 1) * 128] = lo
            wb[:, (2 * j + 1) * 384 + i * 128:(2 * j + 1) * 384 + (i + 1) * 128] = hi
    m_mem.wait(); m_wob.wait()
    r40 = lax.broadcasted_iota(jnp.int32, (40, 40), 0)
    c40 = lax.broadcasted_iota(jnp.int32, (40, 40), 1)
    mask40 = (r40 < NM) | (r40 >= c40)

    def step(s, mem):
        xs = xb_s[pl.ds(pl.multiple_of(s * SEG, SEG), SEG), :].astype(f32)
        hrow = jnp.concatenate([mem, xs], axis=0)
        def qkv(h):
            return jnp.dot(hrow, pltpu.bitcast(wb[:, h * 384:(h + 1) * 384], bf16), preferred_element_type=f32)
        def att(t):
            q = t[:, 0:128] * SCALE
            k = t[:, 128:256].astype(bf16)
            v = t[:, 256:384].astype(bf16)
            sc = lax.dot_general(q, k, NT, preferred_element_type=f32)
            sc = jnp.where(mask40, sc, -1e30)
            m = jnp.max(sc, axis=1, keepdims=True)
            p = jnp.exp2(sc - m)
            l = jnp.sum(p, axis=1, keepdims=True)
            o = jnp.dot(p, v, preferred_element_type=f32)
            return o * (1.0 / l)
        def op(hs, os_):
            o = jnp.concatenate(os_, axis=1) if len(os_) > 1 else os_[0]
            wo = [pltpu.bitcast(wob_s[h * (DM // 2):(h + 1) * (DM // 2), :], bf16) for h in hs]
            wo = jnp.concatenate(wo, axis=1) if len(wo) > 1 else wo[0]
            return lax.dot_general(o, wo, NT, preferred_element_type=f32)
        G = B_G; NG = H // G
        def qkvg(g):
            r = jnp.dot(hrow, pltpu.bitcast(wb[:, g * G * 384:(g + 1) * G * 384], bf16), preferred_element_type=f32)
            return [r[:, i * 384:(i + 1) * 384] for i in range(G)]
        t = {g: qkvg(g) for g in range(min(B_AHEAD, NG))}
        o = {}
        res = None
        for g in range(NG + B_LAG):
            if g + B_AHEAD < NG:
                t[g + B_AHEAD] = qkvg(g + B_AHEAD)
            if g < NG:
                o[g] = [att(x) for x in t.pop(g)]
            gl = g - B_LAG
            if gl >= 0:
                r = op(list(range(gl * G, (gl + 1) * G)), o.pop(gl))
                res = r if res is None else res + r
        out_s[pl.ds(pl.multiple_of(s * SEG, SEG), SEG), DM:2 * DM] = res[NM:].astype(bf16)
        return res[:NM].astype(bf16).astype(f32)
    if do_b:
        lax.fori_loop(0, NSEG, step, mem_s[...].astype(f32))
    else:
        out_s[:, DM:] = jnp.zeros((S, DM), bf16)
    cp = pltpu.make_async_copy(out_s, out_h, sem_o)
    cp.start(); cp.wait()

def run(A_x, A_c_kv, A_w_q, A_w_uk, A_w_uv, A_w_o, B_x, B_mem0, B_Wq, B_Wk, B_Wv, B_Wo, do_a=True, do_b=True):
    anyspec = pl.BlockSpec(memory_space=pltpu.MemorySpace.HBM)
    scratch = [
        pltpu.VMEM((2, DM, S), bf16),
        pltpu.VMEM((S, DM), bf16), pltpu.VMEM((S, DC), bf16), pltpu.VMEM((S, DM), bf16), pltpu.VMEM((NM, DM), bf16),
        pltpu.VMEM((H * DM // 2, D), u32), pltpu.VMEM((H * DM // 2, D), u32),
        pltpu.VMEM((16, DM, D), u32), pltpu.VMEM((16, DC, D), u32), pltpu.VMEM((16, DC, D), u32),
        pltpu.VMEM((16, DM, D), u32), pltpu.VMEM((16, DM, D), u32), pltpu.VMEM((16, DM, D), u32),
        pltpu.VMEM((2, 2, DM // 2, D), u32), pltpu.VMEM((2, 2, DC // 2, 2 * D), u32), pltpu.VMEM((DM // 2, 3 * H * D), u32),
        pltpu.VMEM((S, DM), f32), pltpu.VMEM((S, 2 * DM), bf16),
        pltpu.VMEM((2, S, D), bf16), pltpu.VMEM((2, S, D), bf16), pltpu.VMEM((2, S, D), bf16),
        pltpu.SemaphoreType.DMA((3, 16)), pltpu.SemaphoreType.DMA((3, 16)), pltpu.SemaphoreType.DMA((6,)), pltpu.SemaphoreType.DMA(()),
    ]
    out = pl.pallas_call(
        functools.partial(kernel, do_a=do_a, do_b=do_b),
        out_shape=jax.ShapeDtypeStruct((S, 2 * DM), bf16),
        in_specs=[anyspec] * 12, out_specs=anyspec, scratch_shapes=scratch,
        compiler_params=pltpu.CompilerParams(vmem_limit_bytes=110 * 1024 * 1024),
    )(A_x.reshape(S, DM).T, A_c_kv.reshape(S, DC), A_w_q, A_w_uk, A_w_uv, A_w_o.transpose(0, 2, 1).reshape(H * DM, D),
      B_x.reshape(S, DM).T, B_mem0.reshape(NM, DM), B_Wq, B_Wk, B_Wv, B_Wo.transpose(0, 2, 1).reshape(H * DM, D))
    return out.reshape(1, S, 2 * DM)


@functools.partial(jax.jit, static_argnames=("B_seg_len",))
def pallas_concat_heads__compressed_kv_cla__memory_aug_recurrent_mem_tr__prompt_kernel(A_x, A_c_kv, A_w_q, A_w_uk, A_w_uv, A_w_o, B_x, B_mem0, B_Wq, B_Wk, B_Wv, B_Wo, B_seg_len):
    assert int(B_seg_len) == SEG
    return run(A_x, A_c_kv, A_w_q, A_w_uk, A_w_uv, A_w_o, B_x, B_mem0, B_Wq, B_Wk, B_Wv, B_Wo)
```

```python
import functools
import numpy as np
import jax
import jax.numpy as jnp
from jax import lax
from jax.experimental import pallas as pl
from jax.experimental.pallas import tpu as pltpu

S = 2048; DM = 576; DC = 512; H = 32; D = 128; NM = 8; SEG = 32
NSEG = S // SEG
NOC = 8; OCH = S // NOC
LOG2E = float(np.log2(np.e))
SCALE = float(D ** -0.5) * LOG2E
bf16 = jnp.bfloat16; f32 = jnp.float32; u32 = jnp.uint32
NT = (((1,), (1,)), ((), ()))
B_AHEAD = 2; B_LAG = 4; B_G = 4
A_PCH = 128
A_QKA = 0

def repack(ev, od):
    lo = (ev & u32(0xffff)) | (od << 16)
    hi = (ev >> 16) | (od & u32(0xffff0000))
    return lo, hi

def recip(l):
    r = pl.reciprocal(l, approx=True)
    return r * (2.0 - l * r)

def kernel(xa_h, c_h, wq_h, wuk_h, wuv_h, woa_h, xb_h, mem_h, bq_h, bk_h, bv_h, wob_h, out_h,
           xt_s, xa_s, c_s, xb_s, mem_s, woa_s, wob_s, uq, uk, uv, ubq, ubk, ubv,
           wq_p, wkv_p, wb, acc, out_s, q_s, k_s, v_s, sem_a, sem_b, sem_w, sem_m, sem_o, *, do_a, do_b):
    m_c = pltpu.make_async_copy(c_h, c_s, sem_m.at[0])
    m_xa = pltpu.make_async_copy(xa_h, xt_s.at[0], sem_m.at[1])
    m_xb = pltpu.make_async_copy(xb_h, xt_s.at[1], sem_m.at[3])
    m_mem = pltpu.make_async_copy(mem_h, mem_s, sem_m.at[4])
    m_wob = pltpu.make_async_copy(wob_h.bitcast(u32), wob_s, sem_m.at[5])
    rq, rk, rv = wq_h.bitcast(u32), wuk_h.bitcast(u32), wuv_h.bitcast(u32)
    sq, sk, sv = bq_h.bitcast(u32), bk_h.bitcast(u32), bv_h.bitcast(u32)
    def a_cp(i, j):
        src = (rk, rv, rq)[i]; dst = (uk, uv, uq)[i]
        return pltpu.make_async_copy(src.at[:, j, :], dst.at[j], sem_a.at[i, j])
    woa_u = woa_h.bitcast(u32)
    def wo_cp(j):
        sl = pl.ds(pl.multiple_of(j * DM, DM), DM)
        return pltpu.make_async_copy(woa_u.at[sl, :], woa_s.at[sl, :], sem_w.at[j])
    def b_cp(i, j):
        src = (sq, sk, sv)[i]; dst = (ubq, ubk, ubv)[i]
        return pltpu.make_async_copy(src.at[:, j, :], dst.at[j], sem_b.at[i, j])
    m_c.start()
    a_cp(0, 0).start(); a_cp(1, 0).start()
    m_xa.start()
    a_cp(2, 0).start(); wo_cp(0).start()
    for i in range(3): a_cp(i, 1).start()
    wo_cp(1).start()

    acc[...] = jnp.zeros(acc.shape, f32)
    m_xa.wait()
    for t in range(4):
        xa_s[t * 512:(t + 1) * 512, :] = xt_s[0, :, t * 512:(t + 1) * 512].T
    m_c.wait()
    row = lax.broadcasted_iota(jnp.int32, (128, 128), 0)
    col = lax.broadcasted_iota(jnp.int32, (128, 128), 1)
    tri = row >= col

    def prep_w(j):
        sl = j % 2
        for i in range(3):
            a_cp(i, j).wait()
        lo, hi = repack(uq[j, pl.ds(0, DM // 2, stride=2), :], uq[j, pl.ds(1, DM // 2, stride=2), :])
        wq_p[sl, 0] = lo; wq_p[sl, 1] = hi
        lo, hi = repack(uk[j, pl.ds(0, DC // 2, stride=2), :], uk[j, pl.ds(1, DC // 2, stride=2), :])
        wkv_p[sl, 0, :, 0:128] = lo; wkv_p[sl, 1, :, 0:128] = hi
        lo, hi = repack(uv[j, pl.ds(0, DC // 2, stride=2), :], uv[j, pl.ds(1, DC // 2, stride=2), :])
        wkv_p[sl, 0, :, 128:256] = lo; wkv_p[sl, 1, :, 128:256] = hi

    def proj(sl, hh, r0, n):
        wq = pltpu.bitcast(wq_p[sl, hh], bf16)
        wkv = pltpu.bitcast(wkv_p[sl, hh], bf16)
        kv = jnp.dot(c_s[r0:r0 + n, :], wkv, preferred_element_type=f32)
        k_s[hh, r0:r0 + n, :] = kv[:, 0:128].astype(bf16)
        v_s[hh, r0:r0 + n, :] = kv[:, 128:256].astype(bf16)
        q = jnp.dot(xa_s[r0:r0 + n, :], wq, preferred_element_type=f32) * SCALE
        q_s[hh, r0:r0 + n, :] = q.astype(bf16)

    def qk(hh, qi):
        n = (qi + 1) * 128
        return lax.dot_general(q_s[hh, qi * 128:n, :], k_s[hh, 0:n, :], NT, preferred_element_type=f32)

    def sm_pv(hh, qi, s):
        n = (qi + 1) * 128
        sd = jnp.where(tri, s[:, n - 128:], -1e30)
        s = jnp.concatenate([s[:, :n - 128], sd], axis=1) if qi > 0 else sd
        m = jnp.max(s, axis=1, keepdims=True)
        p = jnp.exp2(s - m)
        l = jnp.sum(p, axis=1, keepdims=True)
        o = jnp.dot(p.astype(bf16), v_s[hh, 0:n, :], preferred_element_type=f32)
        return (o * recip(l)).astype(bf16)

    def oproj(h, qi, ctx):
        w = pltpu.bitcast(woa_s[pl.ds(pl.multiple_of(h * (DM // 2), DM // 2), DM // 2), :], bf16)
        acc[qi * 128:(qi + 1) * 128, :] += lax.dot_general(ctx, w, NT, preferred_element_type=f32)

    def prep_b(j):
        for i, u in enumerate((ubq, ubk, ubv)):
            b_cp(i, j).wait()
            lo, hi = repack(u[j, pl.ds(0, DM // 2, stride=2), :], u[j, pl.ds(1, DM // 2, stride=2), :])
            wb[2 * j, :, i * 128:(i + 1) * 128] = lo
            wb[2 * j + 1, :, i * 128:(i + 1) * 128] = hi
        r0 = pl.multiple_of(j * 128, 128)
        xb_s[pl.ds(r0, 128), :] = xt_s[1, :, pl.ds(r0, 128)].T

    prep_w(0)
    wo_cp(0).wait()
    proj(0, 0, 0, S)

    def pair_body(j, carry):
        sl = j % 2
        jn = jnp.minimum(j + 1, 15)
        @pl.when(j < 14)
        def _():
            for i in range(3): a_cp(i, j + 2).start()
            wo_cp(j + 2).start()
        for i in range(3): b_cp(i, j).start()
        @pl.when(j == 0)
        def _():
            m_xb.start()
        @pl.when(j == 1)
        def _():
            m_mem.start(); m_wob.start()
        @pl.when(j < 15)
        def _():
            prep_w(j + 1)
            wo_cp(j + 1).wait()
        nch = S // A_PCH; every = 16 // nch
        for hh in range(2):
            h = 2 * j + hh
            nsl = sl if hh == 0 else jn % 2
            nh = 1 - hh
            s_cur = qk(hh, 0)
            prev = None
            for qi in range(16):
                if A_QKA and qi < 15:
                    s_next = qk(hh, qi + 1)
                if qi % every == 0:
                    proj(nsl, nh, (qi // every) * A_PCH, A_PCH)
                ctx = sm_pv(hh, qi, s_cur)
                if prev is not None:
                    oproj(h, qi - 1, prev)
                prev = ctx
                if qi < 15:
                    s_cur = s_next if A_QKA else qk(hh, qi + 1)
            oproj(h, 15, prev)
        @pl.when(j == 0)
        def _():
            m_xb.wait()
        prep_b(j)
        return carry
    if do_a:
        lax.fori_loop(0, 16, pair_body, 0)
    else:
        for i in range(3): a_cp(i, 1).wait()
        wo_cp(1).wait()
        m_xb.start(); m_mem.start(); m_wob.start()
        for j in range(16):
            for i in range(3): b_cp(i, j).start()
        m_xb.wait()
        for j in range(16): prep_b(j)
    out_s[:, 0:DM] = acc[...].astype(bf16)

    m_mem.wait(); m_wob.wait()
    r40 = lax.broadcasted_iota(jnp.int32, (40, 40), 0)
    c40 = lax.broadcasted_iota(jnp.int32, (40, 40), 1)
    mask40 = (r40 < NM) | (r40 >= c40)

    def o_cp(c):
        sl = pl.ds(pl.multiple_of(c * OCH, OCH), OCH)
        return pltpu.make_async_copy(out_s.at[sl, :], out_h.at[sl, :], sem_o.at[c])

    def step(s, mem):
        xs = xb_s[pl.ds(pl.multiple_of(s * SEG, SEG), SEG), :].astype(f32)
        hrow = jnp.concatenate([mem, xs], axis=0)
        def qkv(h):
            return jnp.dot(hrow, pltpu.bitcast(wb[:, h * 384:(h + 1) * 384], bf16), preferred_element_type=f32)
        def att(t):
            q = t[:, 0:128] * SCALE
            k = t[:, 128:256].astype(bf16)
            v = t[:, 256:384].astype(bf16)
            sc = lax.dot_general(q, k, NT, preferred_element_type=f32)
            sc = jnp.where(mask40, sc, -1e30)
            m = jnp.max(sc, axis=1, keepdims=True)
            p = jnp.exp2(sc - m)
            l = jnp.sum(p, axis=1, keepdims=True)
            o = jnp.dot(p, v, preferred_element_type=f32)
            return o * recip(l)
        def op(hs, os_):
            o = jnp.concatenate(os_, axis=1) if len(os_) > 1 else os_[0]
            wo = [pltpu.bitcast(wob_s[h * (DM // 2):(h + 1) * (DM // 2), :], bf16) for h in hs]
            wo = jnp.concatenate(wo, axis=1) if len(wo) > 1 else wo[0]
            return lax.dot_general(o, wo, NT, preferred_element_type=f32)
        G = B_G; NG = H // G
        def qkvg(g):
            r = jnp.dot(hrow, jnp.concatenate([pltpu.bitcast(wb[g * G + i], bf16) for i in range(G)], axis=1), preferred_element_type=f32)
            return [r[:, i * 384:(i + 1) * 384] for i in range(G)]
        t = {g: qkvg(g) for g in range(min(B_AHEAD, NG))}
        o = {}
        res = None
        for g in range(NG + B_LAG):
            if g + B_AHEAD < NG:
                t[g + B_AHEAD] = qkvg(g + B_AHEAD)
            if g < NG:
                o[g] = [att(x) for x in t.pop(g)]
            gl = g - B_LAG
            if gl >= 0:
                r = op(list(range(gl * G, (gl + 1) * G)), o.pop(gl))
                res = r if res is None else res + r
        out_s[pl.ds(pl.multiple_of(s * SEG, SEG), SEG), DM:2 * DM] = res[NM:].astype(bf16)
        spc = OCH // SEG
        @pl.when(s % spc == spc - 1)
        def _():
            o_cp(s // spc).start()
        return res[:NM].astype(bf16).astype(f32)
    if do_b:
        lax.fori_loop(0, NSEG, step, mem_s[...].astype(f32))
    else:
        out_s[:, DM:] = jnp.zeros((S, DM), bf16)
        for c in range(NOC): o_cp(c).start()
    for c in range(NOC):
        o_cp(c).wait()

def run(A_x, A_c_kv, A_w_q, A_w_uk, A_w_uv, A_w_o, B_x, B_mem0, B_Wq, B_Wk, B_Wv, B_Wo, do_a=True, do_b=True):
    anyspec = pl.BlockSpec(memory_space=pltpu.MemorySpace.HBM)
    scratch = [
        pltpu.VMEM((2, DM, S), bf16),
        pltpu.VMEM((S, DM), bf16), pltpu.VMEM((S, DC), bf16), pltpu.VMEM((S, DM), bf16), pltpu.VMEM((NM, DM), bf16),
        pltpu.VMEM((H * DM // 2, D), u32), pltpu.VMEM((H * DM // 2, D), u32),
        pltpu.VMEM((16, DM, D), u32), pltpu.VMEM((16, DC, D), u32), pltpu.VMEM((16, DC, D), u32),
        pltpu.VMEM((16, DM, D), u32), pltpu.VMEM((16, DM, D), u32), pltpu.VMEM((16, DM, D), u32),
        pltpu.VMEM((2, 2, DM // 2, D), u32), pltpu.VMEM((2, 2, DC // 2, 2 * D), u32), pltpu.VMEM((H, DM // 2, 3 * D), u32),
        pltpu.VMEM((S, DM), f32), pltpu.VMEM((S, 2 * DM), bf16),
        pltpu.VMEM((2, S, D), bf16), pltpu.VMEM((2, S, D), bf16), pltpu.VMEM((2, S, D), bf16),
        pltpu.SemaphoreType.DMA((3, 16)), pltpu.SemaphoreType.DMA((3, 16)), pltpu.SemaphoreType.DMA((16,)), pltpu.SemaphoreType.DMA((6,)), pltpu.SemaphoreType.DMA((NOC,)),
    ]
    out = pl.pallas_call(
        functools.partial(kernel, do_a=do_a, do_b=do_b),
        out_shape=jax.ShapeDtypeStruct((S, 2 * DM), bf16),
        in_specs=[anyspec] * 12, out_specs=anyspec, scratch_shapes=scratch,
        compiler_params=pltpu.CompilerParams(vmem_limit_bytes=110 * 1024 * 1024),
    )(A_x.reshape(S, DM).T, A_c_kv.reshape(S, DC), A_w_q, A_w_uk, A_w_uv, A_w_o.transpose(0, 2, 1).reshape(H * DM, D),
      B_x.reshape(S, DM).T, B_mem0.reshape(NM, DM), B_Wq, B_Wk, B_Wv, B_Wo.transpose(0, 2, 1).reshape(H * DM, D))
    return out.reshape(1, S, 2 * DM)


@functools.partial(jax.jit, static_argnames=("B_seg_len",))
def pallas_concat_heads__compressed_kv_cla__memory_aug_recurrent_mem_tr__prompt_kernel(A_x, A_c_kv, A_w_q, A_w_uk, A_w_uv, A_w_o, B_x, B_mem0, B_Wq, B_Wk, B_Wv, B_Wo, B_seg_len):
    assert int(B_seg_len) == SEG
    return run(A_x, A_c_kv, A_w_q, A_w_uk, A_w_uv, A_w_o, B_x, B_mem0, B_Wq, B_Wk, B_Wv, B_Wo)
```

```python
import functools
import numpy as np
import jax
import jax.numpy as jnp
from jax import lax
from jax.experimental import pallas as pl
from jax.experimental.pallas import tpu as pltpu

S = 2048; DM = 576; DC = 512; H = 32; D = 128; NM = 8; SEG = 32
NSEG = S // SEG
NOC = 8; OCH = S // NOC
LOG2E = float(np.log2(np.e))
SCALE = float(D ** -0.5) * LOG2E
bf16 = jnp.bfloat16; f32 = jnp.float32; u32 = jnp.uint32
NT = (((1,), (1,)), ((), ()))
B_AHEAD = 2; B_LAG = 4; B_G = 4
A_PCH = 128
A_QKA = 0

def repack(ev, od):
    lo = (ev & u32(0xffff)) | (od << 16)
    hi = (ev >> 16) | (od & u32(0xffff0000))
    return lo, hi

def recip(l):
    r = pl.reciprocal(l, approx=True)
    return r * (2.0 - l * r)

def kernel(xa_h, c_h, wq_h, wuk_h, wuv_h, woa_h, xb_h, mem_h, bq_h, bk_h, bv_h, wob_h, out_h,
           xt_s, xa_s, c_s, xb_s, mem_s, woa_s, wob_s, wob2, uq, uk, uv, ubq, ubk, ubv,
           wq_p, wkv_p, wb, acc, out_s, q_s, k_s, v_s, sem_a, sem_b, sem_w, sem_m, sem_o, *, do_a, do_b):
    m_c = pltpu.make_async_copy(c_h, c_s, sem_m.at[0])
    m_xa = pltpu.make_async_copy(xa_h, xt_s.at[0], sem_m.at[1])
    m_xb = pltpu.make_async_copy(xb_h, xt_s.at[1], sem_m.at[3])
    m_mem = pltpu.make_async_copy(mem_h, mem_s, sem_m.at[4])
    m_wob = pltpu.make_async_copy(wob_h.bitcast(u32), wob_s, sem_m.at[5])
    rq, rk, rv = wq_h.bitcast(u32), wuk_h.bitcast(u32), wuv_h.bitcast(u32)
    sq, sk, sv = bq_h.bitcast(u32), bk_h.bitcast(u32), bv_h.bitcast(u32)
    def a_cp(i, j):
        src = (rk, rv, rq)[i]; dst = (uk, uv, uq)[i]
        return pltpu.make_async_copy(src.at[:, j, :], dst.at[j], sem_a.at[i, j])
    woa_u = woa_h.bitcast(u32)
    def wo_cp(j):
        sl = pl.ds(pl.multiple_of(j * DM, DM), DM)
        return pltpu.make_async_copy(woa_u.at[sl, :], woa_s.at[sl, :], sem_w.at[j])
    def b_cp(i, j):
        src = (sq, sk, sv)[i]; dst = (ubq, ubk, ubv)[i]
        return pltpu.make_async_copy(src.at[:, j, :], dst.at[j], sem_b.at[i, j])
    m_c.start()
    a_cp(0, 0).start(); a_cp(1, 0).start()
    m_xa.start()
    a_cp(2, 0).start(); wo_cp(0).start()
    for i in range(3): a_cp(i, 1).start()
    wo_cp(1).start()

    acc[...] = jnp.zeros(acc.shape, f32)
    m_xa.wait()
    for t in range(4):
        xa_s[t * 512:(t + 1) * 512, :] = xt_s[0, :, t * 512:(t + 1) * 512].T
    m_c.wait()
    row = lax.broadcasted_iota(jnp.int32, (128, 128), 0)
    col = lax.broadcasted_iota(jnp.int32, (128, 128), 1)
    tri = row >= col

    def prep_w(j):
        sl = j % 2
        for i in range(3):
            a_cp(i, j).wait()
        lo, hi = repack(uq[j, pl.ds(0, DM // 2, stride=2), :], uq[j, pl.ds(1, DM // 2, stride=2), :])
        wq_p[sl, 0] = lo; wq_p[sl, 1] = hi
        lo, hi = repack(uk[j, pl.ds(0, DC // 2, stride=2), :], uk[j, pl.ds(1, DC // 2, stride=2), :])
        wkv_p[sl, 0, :, 0:128] = lo; wkv_p[sl, 1, :, 0:128] = hi
        lo, hi = repack(uv[j, pl.ds(0, DC // 2, stride=2), :], uv[j, pl.ds(1, DC // 2, stride=2), :])
        wkv_p[sl, 0, :, 128:256] = lo; wkv_p[sl, 1, :, 128:256] = hi

    def proj(sl, hh, r0, n):
        wq = pltpu.bitcast(wq_p[sl, hh], bf16)
        wkv = pltpu.bitcast(wkv_p[sl, hh], bf16)
        kv = jnp.dot(c_s[r0:r0 + n, :], wkv, preferred_element_type=f32)
        k_s[hh, r0:r0 + n, :] = kv[:, 0:128].astype(bf16)
        v_s[hh, r0:r0 + n, :] = kv[:, 128:256].astype(bf16)
        q = jnp.dot(xa_s[r0:r0 + n, :], wq, preferred_element_type=f32) * SCALE
        q_s[hh, r0:r0 + n, :] = q.astype(bf16)

    def qk(hh, qi):
        n = (qi + 1) * 128
        return lax.dot_general(q_s[hh, qi * 128:n, :], k_s[hh, 0:n, :], NT, preferred_element_type=f32)

    def sm_pv(hh, qi, s):
        n = (qi + 1) * 128
        sd = jnp.where(tri, s[:, n - 128:], -1e30)
        s = jnp.concatenate([s[:, :n - 128], sd], axis=1) if qi > 0 else sd
        m = jnp.max(s, axis=1, keepdims=True)
        p = jnp.exp2(s - m)
        l = jnp.sum(p, axis=1, keepdims=True)
        o = jnp.dot(p.astype(bf16), v_s[hh, 0:n, :], preferred_element_type=f32)
        return (o * recip(l)).astype(bf16)

    def oproj(h, qi, ctx):
        w = pltpu.bitcast(woa_s[pl.ds(pl.multiple_of(h * (DM // 2), DM // 2), DM // 2), :], bf16)
        acc[qi * 128:(qi + 1) * 128, :] += lax.dot_general(ctx, w, NT, preferred_element_type=f32)

    def prep_b(j):
        for i, u in enumerate((ubq, ubk, ubv)):
            b_cp(i, j).wait()
            lo, hi = repack(u[j, pl.ds(0, DM // 2, stride=2), :], u[j, pl.ds(1, DM // 2, stride=2), :])
            wb[2 * j, :, i * 128:(i + 1) * 128] = lo
            wb[2 * j + 1, :, i * 128:(i + 1) * 128] = hi
        r0 = pl.multiple_of(j * 128, 128)
        xb_s[pl.ds(r0, 128), :] = xt_s[1, :, pl.ds(r0, 128)].T

    prep_w(0)
    wo_cp(0).wait()
    proj(0, 0, 0, S)

    def pair_body(j, carry):
        sl = j % 2
        jn = jnp.minimum(j + 1, 15)
        @pl.when(j < 14)
        def _():
            for i in range(3): a_cp(i, j + 2).start()
            wo_cp(j + 2).start()
        for i in range(3): b_cp(i, j).start()
        @pl.when(j == 0)
        def _():
            m_xb.start()
        @pl.when(j == 1)
        def _():
            m_mem.start(); m_wob.start()
        @pl.when(j < 15)
        def _():
            prep_w(j + 1)
            wo_cp(j + 1).wait()
        nch = S // A_PCH; every = 16 // nch
        for hh in range(2):
            h = 2 * j + hh
            nsl = sl if hh == 0 else jn % 2
            nh = 1 - hh
            s_cur = qk(hh, 0)
            prev = None
            for qi in range(16):
                if A_QKA and qi < 15:
                    s_next = qk(hh, qi + 1)
                if qi % every == 0:
                    proj(nsl, nh, (qi // every) * A_PCH, A_PCH)
                ctx = sm_pv(hh, qi, s_cur)
                if prev is not None:
                    oproj(h, qi - 1, prev)
                prev = ctx
                if qi < 15:
                    s_cur = s_next if A_QKA else qk(hh, qi + 1)
            oproj(h, 15, prev)
        @pl.when(j == 0)
        def _():
            m_xb.wait()
        prep_b(j)
        return carry
    if do_a:
        lax.fori_loop(0, 16, pair_body, 0)
    else:
        for i in range(3): a_cp(i, 1).wait()
        wo_cp(1).wait()
        m_xb.start(); m_mem.start(); m_wob.start()
        for j in range(16):
            for i in range(3): b_cp(i, j).start()
        m_xb.wait()
        for j in range(16): prep_b(j)
    out_s[:, 0:DM] = acc[...].astype(bf16)

    m_mem.wait(); m_wob.wait()
    for h in range(H):
        w = pltpu.bitcast(wob_s[h * (DM // 2):(h + 1) * (DM // 2), :], bf16)
        wob2[h] = pltpu.bitcast(w.T, u32)
    r40 = lax.broadcasted_iota(jnp.int32, (40, 40), 0)
    c40 = lax.broadcasted_iota(jnp.int32, (40, 40), 1)
    mask40 = (r40 < NM) | (r40 >= c40)

    def o_cp(c):
        sl = pl.ds(pl.multiple_of(c * OCH, OCH), OCH)
        return pltpu.make_async_copy(out_s.at[sl, :], out_h.at[sl, :], sem_o.at[c])

    def step(s, mem):
        xs = xb_s[pl.ds(pl.multiple_of(s * SEG, SEG), SEG), :].astype(f32)
        hrow = jnp.concatenate([mem, xs], axis=0)
        def qkv(h):
            return jnp.dot(hrow, pltpu.bitcast(wb[:, h * 384:(h + 1) * 384], bf16), preferred_element_type=f32)
        def att(t):
            q = t[:, 0:128] * SCALE
            k = t[:, 128:256].astype(bf16)
            v = t[:, 256:384].astype(bf16)
            sc = lax.dot_general(q, k, NT, preferred_element_type=f32)
            sc = jnp.where(mask40, sc, -1e30)
            m = jnp.max(sc, axis=1, keepdims=True)
            p = jnp.exp2(sc - m)
            l = jnp.sum(p, axis=1, keepdims=True)
            o = jnp.dot(p, v, preferred_element_type=f32)
            return o * recip(l)
        def op(hs, os_):
            o = jnp.concatenate(os_, axis=1) if len(os_) > 1 else os_[0]
            wo = [pltpu.bitcast(wob2[h], bf16) for h in hs]
            wo = jnp.concatenate(wo, axis=0) if len(wo) > 1 else wo[0]
            return jnp.dot(o, wo, preferred_element_type=f32)
        G = B_G; NG = H // G
        def qkvg(g):
            r = jnp.dot(hrow, jnp.concatenate([pltpu.bitcast(wb[g * G + i], bf16) for i in range(G)], axis=1), preferred_element_type=f32)
            return [r[:, i * 384:(i + 1) * 384] for i in range(G)]
        t = {g: qkvg(g) for g in range(min(B_AHEAD, NG))}
        o = {}
        res = None
        for g in range(NG + B_LAG):
            if g + B_AHEAD < NG:
                t[g + B_AHEAD] = qkvg(g + B_AHEAD)
            if g < NG:
                o[g] = [att(x) for x in t.pop(g)]
            gl = g - B_LAG
            if gl >= 0:
                r = op(list(range(gl * G, (gl + 1) * G)), o.pop(gl))
                res = r if res is None else res + r
        out_s[pl.ds(pl.multiple_of(s * SEG, SEG), SEG), DM:2 * DM] = res[NM:].astype(bf16)
        spc = OCH // SEG
        @pl.when(s % spc == spc - 1)
        def _():
            o_cp(s // spc).start()
        return res[:NM].astype(bf16).astype(f32)
    if do_b:
        lax.fori_loop(0, NSEG, step, mem_s[...].astype(f32))
    else:
        out_s[:, DM:] = jnp.zeros((S, DM), bf16)
        for c in range(NOC): o_cp(c).start()
    for c in range(NOC):
        o_cp(c).wait()

def run(A_x, A_c_kv, A_w_q, A_w_uk, A_w_uv, A_w_o, B_x, B_mem0, B_Wq, B_Wk, B_Wv, B_Wo, do_a=True, do_b=True):
    anyspec = pl.BlockSpec(memory_space=pltpu.MemorySpace.HBM)
    scratch = [
        pltpu.VMEM((2, DM, S), bf16),
        pltpu.VMEM((S, DM), bf16), pltpu.VMEM((S, DC), bf16), pltpu.VMEM((S, DM), bf16), pltpu.VMEM((NM, DM), bf16),
        pltpu.VMEM((H * DM // 2, D), u32), pltpu.VMEM((H * DM // 2, D), u32), pltpu.VMEM((H, D // 2, DM), u32),
        pltpu.VMEM((16, DM, D), u32), pltpu.VMEM((16, DC, D), u32), pltpu.VMEM((16, DC, D), u32),
        pltpu.VMEM((16, DM, D), u32), pltpu.VMEM((16, DM, D), u32), pltpu.VMEM((16, DM, D), u32),
        pltpu.VMEM((2, 2, DM // 2, D), u32), pltpu.VMEM((2, 2, DC // 2, 2 * D), u32), pltpu.VMEM((H, DM // 2, 3 * D), u32),
        pltpu.VMEM((S, DM), f32), pltpu.VMEM((S, 2 * DM), bf16),
        pltpu.VMEM((2, S, D), bf16), pltpu.VMEM((2, S, D), bf16), pltpu.VMEM((2, S, D), bf16),
        pltpu.SemaphoreType.DMA((3, 16)), pltpu.SemaphoreType.DMA((3, 16)), pltpu.SemaphoreType.DMA((16,)), pltpu.SemaphoreType.DMA((6,)), pltpu.SemaphoreType.DMA((NOC,)),
    ]
    out = pl.pallas_call(
        functools.partial(kernel, do_a=do_a, do_b=do_b),
        out_shape=jax.ShapeDtypeStruct((S, 2 * DM), bf16),
        in_specs=[anyspec] * 12, out_specs=anyspec, scratch_shapes=scratch,
        compiler_params=pltpu.CompilerParams(vmem_limit_bytes=110 * 1024 * 1024),
    )(A_x.reshape(S, DM).T, A_c_kv.reshape(S, DC), A_w_q, A_w_uk, A_w_uv, A_w_o.transpose(0, 2, 1).reshape(H * DM, D),
      B_x.reshape(S, DM).T, B_mem0.reshape(NM, DM), B_Wq, B_Wk, B_Wv, B_Wo.transpose(0, 2, 1).reshape(H * DM, D))
    return out.reshape(1, S, 2 * DM)


@functools.partial(jax.jit, static_argnames=("B_seg_len",))
def pallas_concat_heads__compressed_kv_cla__memory_aug_recurrent_mem_tr__prompt_kernel(A_x, A_c_kv, A_w_q, A_w_uk, A_w_uv, A_w_o, B_x, B_mem0, B_Wq, B_Wk, B_Wv, B_Wo, B_seg_len):
    assert int(B_seg_len) == SEG
    return run(A_x, A_c_kv, A_w_q, A_w_uk, A_w_uv, A_w_o, B_x, B_mem0, B_Wq, B_Wk, B_Wv, B_Wo)
```
